```python
import os as _os
_os.environ.setdefault("JAX_PLATFORMS", "cpu")
import jax
import jax.numpy as jnp

def _softmax(x, axis=-1):
    return jax.nn.softmax(x, axis=axis)
def _gelu(x):
    return jax.nn.gelu(x, approximate=True)
def _silu(x):
    return jax.nn.silu(x)
def _sigmoid(x):
    return jax.nn.sigmoid(x)
def _layernorm(x, axis=-1, eps=1e-5):
    m = jnp.mean(x, axis=axis, keepdims=True)
    v = jnp.var(x, axis=axis, keepdims=True)
    return (x - m) / jnp.sqrt(v + eps)
def _scatter_add(tgt, idx, src, axis=0):
    return tgt.at[idx].add(src)
def _segment_sum(src, seg, n):
    return jax.ops.segment_sum(src, seg, n)
class _Rng:
    def __init__(self, key):
        self._k = key
    def _next(self):
        self._k, sub = jax.random.split(self._k)
        return sub
    def normal(self, shape):
        return jax.random.normal(self._next(), shape, dtype=jnp.bfloat16)
    def randint(self, lo, hi, shape):
        return jax.random.randint(self._next(), shape, lo, hi, dtype=jnp.int32)
    def uniform(self, shape, lo=0.0, hi=1.0):
        return jax.random.uniform(self._next(), shape, jnp.bfloat16, lo, hi)
    def permutation(self, n):
        return jax.random.permutation(self._next(), n)


kernel_name = 'standalone__gqa_block_cached__near_ridge'

def setup_inputs():
    _rng = _Rng(jax.random.key(int.from_bytes(__import__("os").urandom(4), "little")))
    _w = (lambda a: (lambda t: t.astype(jnp.bfloat16) if jnp.issubdtype(t.dtype, jnp.floating) else t)(jnp.asarray(a)))
    B, Sq, D = 8, 96, 640
    Hq, Hkv, Sk, Dh = 32, 32, 512, 128
    assert Hq % Hkv == 0, (Hq, Hkv)
    return {
        "x": _w((lambda *s: _rng.normal(s) * 0.2)(B, Sq, D)),
        "k_cache": _w((lambda *s: _rng.normal(s) * 3.2)(B, Hkv, Sk, Dh)),
        "v_cache": _w((lambda *s: _rng.normal(s) * 0.05)(B, Hkv, Sk, Dh)),
        "wq": _w((lambda *s: _rng.normal(s) * 0.2)(D, Hq * Dh) * (D ** -0.5)),
        "wo": _w((lambda *s: _rng.normal(s) * 0.05)(Hq * Dh, D) * ((Hq * Dh) ** -0.5)),
    }

def reference(x, k_cache, v_cache, wq, wo):
    B, Sq, D = x.shape
    Hq, Dh = 32, 128
    Hkv = k_cache.shape[1]
    rep = Hq // Hkv
    q = (lambda x, *d: x.transpose(*d))((x @ wq).reshape(B, Sq, Hq, Dh), 0, 2, 1, 3)
    k = jnp.repeat(k_cache, rep, axis=1)
    v = jnp.repeat(v_cache, rep, axis=1)
    scores = jnp.einsum("bhqd,bhkd->bhqk", q, k) * (Dh ** -0.5)
    p = _softmax(scores, axis=-1)
    o = jnp.einsum("bhqk,bhkd->bhqd", p, v)
    return (lambda x, *d: x.transpose(*d))(o, 0, 2, 1, 3).reshape(B, Sq, Hq * Dh) @ wo
```

```python
import functools

import jax
import jax.numpy as jnp
import jax.experimental.pallas as pl
import jax.experimental.pallas.tpu as pltpu


@jax.jit
def pallas_standalone__gqa_block_cached__near_ridge_kernel(
    x: jax.Array,
    k_cache: jax.Array,
    v_cache: jax.Array,
    wq: jax.Array,
    wo: jax.Array,
):
    B, Sq, D = x.shape
    _, Hkv, Sk, Dh = k_cache.shape
    Hq = wq.shape[1] // Dh
    rep = Hq // Hkv
    M = B * Sq
    scale = Dh ** -0.5

    x2 = x.reshape(M, D)

    def kernel_function(x_ref, k_ref, v_ref, wq_ref, wo_ref, out_ref, acc_ref, o_ref):
        h = pl.program_id(0)

        q = jnp.dot(x_ref[...], wq_ref[...], preferred_element_type=jnp.float32)
        q = (q * scale).astype(jnp.bfloat16)
        for b in range(B):
            qb = q[b * Sq:(b + 1) * Sq]
            s = jax.lax.dot_general(qb, k_ref[b, 0], (((1,), (1,)), ((), ())),
                                    preferred_element_type=jnp.float32)
            m = jnp.max(s, axis=-1, keepdims=True)
            p = jnp.exp(s - m)
            l = jnp.sum(p, axis=-1, keepdims=True)
            o = jnp.dot(p.astype(jnp.bfloat16), v_ref[b, 0],
                        preferred_element_type=jnp.float32)
            o_ref[b * Sq:(b + 1) * Sq, :] = (o / l).astype(jnp.bfloat16)
        contrib = jnp.dot(o_ref[...], wo_ref[...], preferred_element_type=jnp.float32)

        @pl.when(h == 0)
        def _():
            acc_ref[...] = contrib

        @pl.when(h > 0)
        def _():
            acc_ref[...] += contrib

        @pl.when(h == Hq - 1)
        def _():
            out_ref[...] = acc_ref[...].astype(out_ref.dtype)

    out = pl.pallas_call(
        kernel_function,
        grid=(Hq,),
        in_specs=[
            pl.BlockSpec((M, D), lambda h: (0, 0)),
            pl.BlockSpec((B, 1, Sk, Dh), lambda h: (0, h // rep, 0, 0)),
            pl.BlockSpec((B, 1, Sk, Dh), lambda h: (0, h // rep, 0, 0)),
            pl.BlockSpec((D, Dh), lambda h: (0, h)),
            pl.BlockSpec((Dh, D), lambda h: (h, 0)),
        ],
        out_specs=pl.BlockSpec((M, D), lambda h: (0, 0)),
        out_shape=jax.ShapeDtypeStruct((M, D), x.dtype),
        scratch_shapes=[
            pltpu.VMEM((M, D), jnp.float32),
            pltpu.VMEM((M, Dh), jnp.bfloat16),
        ],
        compiler_params=pltpu.CompilerParams(
            dimension_semantics=("arbitrary",),
            vmem_limit_bytes=64 * 1024 * 1024,
        ),
    )(x2, k_cache, v_cache, wq, wo)
    return out.reshape(B, Sq, D)
```

```python
import jax
import jax.numpy as jnp
import jax.experimental.pallas as pl
import jax.experimental.pallas.tpu as pltpu


@jax.jit
def pallas_standalone__gqa_block_cached__near_ridge_kernel(
    x: jax.Array,
    k_cache: jax.Array,
    v_cache: jax.Array,
    wq: jax.Array,
    wo: jax.Array,
):
    B, Sq, D = x.shape
    _, Hkv, Sk, Dh = k_cache.shape
    Hq = wq.shape[1] // Dh
    rep = Hq // Hkv
    M = B * Sq
    scale = Dh ** -0.5

    CB = 2 if B % 2 == 0 else 1
    NC = B // CB
    R = CB * Sq
    T = CB
    B1 = B - T
    assert B1 > 0 and B1 % CB == 0
    NC1 = B1 // CB
    last = Hkv - 1

    x2 = x.reshape(M, D)

    def kernel_function(x_ref, k_hbm, v_hbm, wq_ref, wo_ref, out_hbm,
                        acc_ref, o_ref, q_ref, kbuf, vbuf, obuf, ksem, vsem, osem):
        g = pl.program_id(0)
        slot = g % 2

        def kv_copies(head, s, b0, n):
            return (
                pltpu.make_async_copy(k_hbm.at[pl.ds(b0, n), head],
                                      kbuf.at[s, pl.ds(b0, n)], ksem.at[s]),
                pltpu.make_async_copy(v_hbm.at[pl.ds(b0, n), head],
                                      vbuf.at[s, pl.ds(b0, n)], vsem.at[s]),
            )

        def o_copy(i, r0, n):
            return pltpu.make_async_copy(obuf.at[pl.ds(r0, n)],
                                         out_hbm.at[pl.ds(r0, n)], osem.at[i])

        @pl.when(g == 0)
        def _():
            for c in kv_copies(0, 0, 0, B if last > 0 else B1):
                c.start()
            acc_ref[...] = jnp.zeros_like(acc_ref)

        @pl.when(g + 1 < last)
        def _():
            for c in kv_copies(g + 1, 1 - slot, 0, B):
                c.start()

        @pl.when(g + 1 == last)
        def _():
            for c in kv_copies(last, 1 - slot, 0, B1):
                c.start()

        @pl.when(g == last)
        def _():
            for c in kv_copies(last, 1 - slot, B1, T):
                c.start()

        @pl.when(g < last)
        def _():
            for c in kv_copies(g, slot, 0, B):
                c.wait()

        @pl.when(g == last)
        def _():
            for c in kv_copies(last, slot, 0, B1):
                c.wait()

        @pl.when(g == last + 1)
        def _():
            for c in kv_copies(last, slot, B1, T):
                c.wait()

        def qproj(r, c):
            q = jnp.dot(x_ref[c * R:(c + 1) * R, :], wq_ref[:, r * Dh:(r + 1) * Dh],
                        preferred_element_type=jnp.float32)
            q_ref[r, c * R:(c + 1) * R, :] = (q * scale).astype(q_ref.dtype)

        def oproj(r, c):
            acc_ref[c * R:(c + 1) * R, :] += jnp.dot(
                o_ref[c * R:(c + 1) * R, :], wo_ref[r * Dh:(r + 1) * Dh, :],
                preferred_element_type=jnp.float32)

        def qk(r, b):
            return jax.lax.dot_general(q_ref[r, b * Sq:(b + 1) * Sq, :], kbuf[slot, b],
                                       (((1,), (1,)), ((), ())),
                                       preferred_element_type=jnp.float32)

        def attend(r, b0, b1, do_qproj, extra_qproj):
            c0, c1 = b0 // CB, b1 // CB
            if do_qproj:
                qproj(r, c0)
            s_next = qk(r, b0)
            for b in range(b0, b1):
                c = b // CB
                if b % CB == 0:
                    if do_qproj and c + 1 < c1 + extra_qproj:
                        qproj(r, c + 1)
                    if c - 1 >= c0:
                        oproj(r, c - 1)
                s = s_next
                if b + 1 < b1:
                    s_next = qk(r, b + 1)
                m = jnp.max(s, axis=-1, keepdims=True)
                p = jnp.exp(s - m)
                l = jnp.sum(p, axis=-1, keepdims=True)
                o = jnp.dot(p.astype(vbuf.dtype), vbuf[slot, b],
                            preferred_element_type=jnp.float32)
                o_ref[b * Sq:(b + 1) * Sq, :] = (o / l).astype(o_ref.dtype)
            for c in range(c1 + 1, c1 + extra_qproj):
                qproj(r, c)
            oproj(r, c1 - 1)

        @pl.when(g < last)
        def _():
            for r in range(rep):
                attend(r, 0, B, True, 0)

        @pl.when(g == last)
        def _():
            for r in range(rep):
                attend(r, 0, B1, True, NC - NC1)
            obuf[0:B1 * Sq, :] = acc_ref[0:B1 * Sq, :].astype(obuf.dtype)
            o_copy(0, 0, B1 * Sq).start()

        @pl.when(g == last + 1)
        def _():
            for r in range(rep):
                attend(r, B1, B, False, 0)
            obuf[B1 * Sq:M, :] = acc_ref[B1 * Sq:M, :].astype(obuf.dtype)
            o_copy(1, B1 * Sq, T * Sq).start()
            o_copy(0, 0, B1 * Sq).wait()
            o_copy(1, B1 * Sq, T * Sq).wait()

    out = pl.pallas_call(
        kernel_function,
        grid=(Hkv + 1,),
        in_specs=[
            pl.BlockSpec((M, D), lambda g: (0, 0)),
            pl.BlockSpec(memory_space=pl.ANY),
            pl.BlockSpec(memory_space=pl.ANY),
            pl.BlockSpec((D, rep * Dh), lambda g: (0, jnp.minimum(g, last))),
            pl.BlockSpec((rep * Dh, D), lambda g: (jnp.minimum(g, last), 0)),
        ],
        out_specs=pl.BlockSpec(memory_space=pl.ANY),
        out_shape=jax.ShapeDtypeStruct((M, D), x.dtype),
        scratch_shapes=[
            pltpu.VMEM((M, D), jnp.float32),
            pltpu.VMEM((M, Dh), jnp.bfloat16),
            pltpu.VMEM((rep, M, Dh), jnp.bfloat16),
            pltpu.VMEM((2, B, Sk, Dh), k_cache.dtype),
            pltpu.VMEM((2, B, Sk, Dh), v_cache.dtype),
            pltpu.VMEM((M, D), x.dtype),
            pltpu.SemaphoreType.DMA((2,)),
            pltpu.SemaphoreType.DMA((2,)),
            pltpu.SemaphoreType.DMA((2,)),
        ],
        compiler_params=pltpu.CompilerParams(
            dimension_semantics=("arbitrary",),
            vmem_limit_bytes=64 * 1024 * 1024,
        ),
    )(x2, k_cache, v_cache, wq, wo)
    return out.reshape(B, Sq, D)
```

```python
import jax
import jax.numpy as jnp
import jax.experimental.pallas as pl
import jax.experimental.pallas.tpu as pltpu


@jax.jit
def pallas_standalone__gqa_block_cached__near_ridge_kernel(
    x: jax.Array,
    k_cache: jax.Array,
    v_cache: jax.Array,
    wq: jax.Array,
    wo: jax.Array,
):
    B, Sq, D = x.shape
    _, Hkv, Sk, Dh = k_cache.shape
    Hq = wq.shape[1] // Dh
    rep = Hq // Hkv
    M = B * Sq
    scale = Dh ** -0.5

    CB = 2 if B % 2 == 0 else 1
    NC = B // CB
    R = CB * Sq
    T = CB
    B1 = B - T
    assert B1 > 0 and B1 % CB == 0
    last = Hkv - 1

    x2 = x.reshape(M, D)

    def kernel_function(x_ref, k_hbm, v_hbm, wq0_ref, wq_ref, wo_ref, out_hbm,
                        acc_ref, o_ref, qc_ref, qn_ref, kbuf, vbuf, obuf,
                        ksem, vsem, osem):
        g = pl.program_id(0)
        slot = g % 2

        def kv_copies(head, s, b0, n):
            return (
                pltpu.make_async_copy(k_hbm.at[pl.ds(b0, n), head],
                                      kbuf.at[s, pl.ds(b0, n)], ksem.at[s]),
                pltpu.make_async_copy(v_hbm.at[pl.ds(b0, n), head],
                                      vbuf.at[s, pl.ds(b0, n)], vsem.at[s]),
            )

        def o_copy(i, r0, n):
            return pltpu.make_async_copy(obuf.at[pl.ds(r0, n)],
                                         out_hbm.at[pl.ds(r0, n)], osem.at[i])

        def qproj(w_ref, r, c):
            q = jnp.dot(x_ref[c * R:(c + 1) * R, :], w_ref[:, r * Dh:(r + 1) * Dh],
                        preferred_element_type=jnp.float32)
            qn_ref[r, c * R:(c + 1) * R, :] = (q * scale).astype(qn_ref.dtype)

        @pl.when(g == 0)
        def _():
            for c in kv_copies(0, 0, 0, B if last > 0 else B1):
                c.start()

        @pl.when(g + 1 < last)
        def _():
            for c in kv_copies(g + 1, 1 - slot, 0, B):
                c.start()

        @pl.when(g + 1 == last)
        def _():
            for c in kv_copies(last, 1 - slot, 0, B1):
                c.start()

        @pl.when(g == last)
        def _():
            for c in kv_copies(last, 1 - slot, B1, T):
                c.start()

        @pl.when(g == 0)
        def _():
            acc_ref[...] = jnp.zeros_like(acc_ref)
            for r in range(rep):
                for c in range(NC):
                    qproj(wq0_ref, r, c)

        @pl.when(g < last)
        def _():
            for c in kv_copies(g, slot, 0, B):
                c.wait()

        @pl.when(g == last)
        def _():
            for c in kv_copies(last, slot, 0, B1):
                c.wait()

        @pl.when(g == last + 1)
        def _():
            for c in kv_copies(last, slot, B1, T):
                c.wait()

        def oproj(r, c):
            acc_ref[c * R:(c + 1) * R, :] += jnp.dot(
                o_ref[c * R:(c + 1) * R, :], wo_ref[r * Dh:(r + 1) * Dh, :],
                preferred_element_type=jnp.float32)

        def qk(r, b):
            return jax.lax.dot_general(qc_ref[r, b * Sq:(b + 1) * Sq, :], kbuf[slot, b],
                                       (((1,), (1,)), ((), ())),
                                       preferred_element_type=jnp.float32)

        def attend(r, b0, b1, do_qproj):
            c0, c1 = b0 // CB, b1 // CB
            s_next = qk(r, b0)
            for b in range(b0, b1):
                c = b // CB
                if b % CB == 0:
                    if do_qproj:
                        qproj(wq_ref, r, c)
                    if c - 1 >= c0:
                        oproj(r, c - 1)
                s = s_next
                if b + 1 < b1:
                    s_next = qk(r, b + 1)
                m = jnp.max(s, axis=-1, keepdims=True)
                p = jnp.exp(s - m)
                l = jnp.sum(p, axis=-1, keepdims=True)
                o = jnp.dot(p.astype(vbuf.dtype), vbuf[slot, b],
                            preferred_element_type=jnp.float32)
                o_ref[b * Sq:(b + 1) * Sq, :] = (o / l).astype(o_ref.dtype)
            oproj(r, c1 - 1)

        @pl.when(g < last)
        def _():
            qc_ref[...] = qn_ref[...]
            for r in range(rep):
                attend(r, 0, B, True)

        @pl.when(g == last)
        def _():
            qc_ref[...] = qn_ref[...]
            for r in range(rep):
                attend(r, 0, B1, False)
            obuf[0:B1 * Sq, :] = acc_ref[0:B1 * Sq, :].astype(obuf.dtype)
            o_copy(0, 0, B1 * Sq).start()

        @pl.when(g == last + 1)
        def _():
            for r in range(rep):
                attend(r, B1, B, False)
            obuf[B1 * Sq:M, :] = acc_ref[B1 * Sq:M, :].astype(obuf.dtype)
            o_copy(1, B1 * Sq, T * Sq).start()
            o_copy(0, 0, B1 * Sq).wait()
            o_copy(1, B1 * Sq, T * Sq).wait()

    out = pl.pallas_call(
        kernel_function,
        grid=(Hkv + 1,),
        in_specs=[
            pl.BlockSpec((M, D), lambda g: (0, 0)),
            pl.BlockSpec(memory_space=pl.ANY),
            pl.BlockSpec(memory_space=pl.ANY),
            pl.BlockSpec((D, rep * Dh), lambda g: (0, 0)),
            pl.BlockSpec((D, rep * Dh), lambda g: (0, jnp.minimum(g + 1, last))),
            pl.BlockSpec((rep * Dh, D), lambda g: (jnp.minimum(g, last), 0)),
        ],
        out_specs=pl.BlockSpec(memory_space=pl.ANY),
        out_shape=jax.ShapeDtypeStruct((M, D), x.dtype),
        scratch_shapes=[
            pltpu.VMEM((M, D), jnp.float32),
            pltpu.VMEM((M, Dh), jnp.bfloat16),
            pltpu.VMEM((rep, M, Dh), jnp.bfloat16),
            pltpu.VMEM((rep, M, Dh), jnp.bfloat16),
            pltpu.VMEM((2, B, Sk, Dh), k_cache.dtype),
            pltpu.VMEM((2, B, Sk, Dh), v_cache.dtype),
            pltpu.VMEM((M, D), x.dtype),
            pltpu.SemaphoreType.DMA((2,)),
            pltpu.SemaphoreType.DMA((2,)),
            pltpu.SemaphoreType.DMA((2,)),
        ],
        compiler_params=pltpu.CompilerParams(
            dimension_semantics=("arbitrary",),
            vmem_limit_bytes=64 * 1024 * 1024,
        ),
    )(x2, k_cache, v_cache, wq, wq, wo)
    return out.reshape(B, Sq, D)
```
